```python
import os as _os
_os.environ.setdefault("JAX_PLATFORMS", "cpu")
import jax
import jax.numpy as jnp

def _softmax(x, axis=-1):
    return jax.nn.softmax(x, axis=axis)
def _gelu(x):
    return jax.nn.gelu(x, approximate=True)
def _silu(x):
    return jax.nn.silu(x)
def _sigmoid(x):
    return jax.nn.sigmoid(x)
def _layernorm(x, axis=-1, eps=1e-5):
    m = jnp.mean(x, axis=axis, keepdims=True)
    v = jnp.var(x, axis=axis, keepdims=True)
    return (x - m) / jnp.sqrt(v + eps)
def _scatter_add(tgt, idx, src, axis=0):
    return tgt.at[idx].add(src)
def _segment_sum(src, seg, n):
    return jax.ops.segment_sum(src, seg, n)
class _Rng:
    def __init__(self, key):
        self._k = key
    def _next(self):
        self._k, sub = jax.random.split(self._k)
        return sub
    def normal(self, shape):
        return jax.random.normal(self._next(), shape, dtype=jnp.bfloat16)
    def randint(self, lo, hi, shape):
        return jax.random.randint(self._next(), shape, lo, hi, dtype=jnp.int32)
    def uniform(self, shape, lo=0.0, hi=1.0):
        return jax.random.uniform(self._next(), shape, jnp.bfloat16, lo, hi)
    def permutation(self, n):
        return jax.random.permutation(self._next(), n)


kernel_name = 'standalone__layernorm_linear__sampling'

def setup_inputs():
    _rng = _Rng(jax.random.key(int.from_bytes(__import__("os").urandom(4), "little")))
    _w = (lambda a: (lambda t: t.astype(jnp.bfloat16) if jnp.issubdtype(t.dtype, jnp.floating) else t)(jnp.asarray(a)))
    B, S, D = 1024, 32, 576
    return {
        "x": _w((lambda *s: _rng.normal(s) * 0.05)(B, S, D)),
        "g": _w((lambda *s: _rng.normal(s) * 0.05)(D) + 1.0),
        "b": _w((lambda *s: _rng.normal(s) * 0.05)(D)),
        "w": _w((lambda *s: _rng.normal(s) * 0.05)(D, D)),
    }

def reference(x, g, b, w):
    return (_layernorm(x, axis=-1) * g + b) @ w
```

```python
import jax
import jax.numpy as jnp
import jax.experimental.pallas as pl
import jax.experimental.pallas.tpu as pltpu

SB = 1
TB = 1024
XPOSE = 'xlu'

@jax.jit
def pallas_standalone__layernorm_linear__sampling_kernel(x, g, b, w):
    B, S, D = x.shape
    xt = jnp.transpose(x, (1, 2, 0))
    g2 = g.reshape(1, D)
    b2 = b.reshape(1, D)
    f32 = jnp.float32

    def kernel(x_ref, g_ref, b_ref, w_ref, o_ref, wt_ref, s_ref, c_ref):
        @pl.when(jnp.logical_and(pl.program_id(0) == 0, pl.program_id(1) == 0))
        def _():
            if XPOSE == 'xlu':
                wt = w_ref[...].astype(f32).T
            else:
                eye = (jax.lax.broadcasted_iota(jnp.int32, (D, D), 0)
                       == jax.lax.broadcasted_iota(jnp.int32, (D, D), 1)).astype(jnp.bfloat16)
                wt = jax.lax.dot_general(eye, w_ref[...], (((1,), (1,)), ((), ())),
                                         preferred_element_type=f32)
            wg = (wt * g_ref[...].astype(f32)).astype(jnp.bfloat16)
            wt_ref[...] = wg
            s = jnp.sum(wg.astype(f32), axis=1, keepdims=True)
            c = jnp.sum(wt * b_ref[...].astype(f32), axis=1, keepdims=True)
            s_ref[...] = jnp.broadcast_to(s, (D, 128))
            c_ref[...] = jnp.broadcast_to(c, (D, 128))

        for si in range(SB):
            xb = x_ref[si]
            acc = jnp.dot(wt_ref[...], xb, preferred_element_type=f32)
            xf = xb.astype(f32)
            m = jnp.sum(xf, axis=0, keepdims=True) * (1.0 / D)
            xc = xf - m
            v = jnp.sum(xc * xc, axis=0, keepdims=True) * (1.0 / D)
            r = jax.lax.rsqrt(v + 1e-5)
            s = jnp.tile(s_ref[...], (1, TB // 128))
            c = jnp.tile(c_ref[...], (1, TB // 128))
            o_ref[si] = ((acc - s * m) * r + c).astype(o_ref.dtype)

    out = pl.pallas_call(
        kernel,
        grid=(S // SB, B // TB),
        in_specs=[
            pl.BlockSpec((SB, D, TB), lambda s, j: (s, 0, j)),
            pl.BlockSpec((1, D), lambda s, j: (0, 0)),
            pl.BlockSpec((1, D), lambda s, j: (0, 0)),
            pl.BlockSpec((D, D), lambda s, j: (0, 0)),
        ],
        out_specs=pl.BlockSpec((SB, D, TB), lambda s, j: (s, 0, j)),
        out_shape=jax.ShapeDtypeStruct((S, D, B), x.dtype),
        scratch_shapes=[pltpu.VMEM((D, D), jnp.bfloat16),
                        pltpu.VMEM((D, 128), f32),
                        pltpu.VMEM((D, 128), f32)],
        compiler_params=pltpu.CompilerParams(
            dimension_semantics=("arbitrary", "arbitrary"),
            vmem_limit_bytes=64 * 1024 * 1024),
    )(xt, g2, b2, w)
    return jnp.transpose(out, (2, 0, 1))
```

```python
import jax
import jax.numpy as jnp
import jax.experimental.pallas as pl
import jax.experimental.pallas.tpu as pltpu

SB = 1
RPI = 3
LOOK = 2
WSTART = 8
NOBC = True
NORM_T0, NORM_T1 = 0, 56
STAT_T0, STAT_T1 = 0, 76

@jax.jit
def pallas_standalone__layernorm_linear__sampling_kernel(x, g, b, w):
    B, S, D = x.shape
    xt = jnp.transpose(x, (1, 2, 0))
    f32, bf16, u32 = jnp.float32, jnp.bfloat16, jnp.uint32
    NIT = S // SB
    HT = 128
    QT = 2 * HT
    NQ = B // QT
    NU = NQ * SB
    KH, MH = 256, D // 2
    KM = 2 * KH
    KR = D - KM
    NR = MH // 16

    def pk(t):
        return pltpu.bitcast(t, u32)

    def upk(t):
        return pltpu.bitcast(t, bf16)

    def kernel(x_hbm, g_hbm, b_hbm, w_hbm, o_hbm,
               xbuf, obuf, w_ref, g_ref, b_ref, a_ref, ar_ref, c_ref, bb_ref, st_ref,
               sem_in, sem_out, sem_p):
        def in_copy(s):
            return pltpu.make_async_copy(x_hbm.at[s], xbuf.at[s], sem_in.at[s])

        def out_copy(s):
            return pltpu.make_async_copy(obuf.at[s], o_hbm.at[s], sem_out.at[s])

        cw = pltpu.make_async_copy(w_hbm, w_ref, sem_p.at[0])
        cg = pltpu.make_async_copy(g_hbm, g_ref, sem_p.at[1])
        cb = pltpu.make_async_copy(b_hbm, b_ref, sem_p.at[2])
        cw.start(); cg.start(); cb.start()
        in_copy(0).start()
        cw.wait(); cg.wait(); cb.wait()
        for t in range(1, LOOK):
            in_copy(t).start()

        wt = w_ref[...].astype(f32).T
        gr = g_ref[...].astype(f32).reshape(1, D)
        br = b_ref[...].astype(f32).reshape(1, D)
        a = wt * gr
        a11, a12 = a[:MH, :KH], a[:MH, KH:KM]
        a21, a22 = a[MH:, :KH], a[MH:, KH:KM]
        for i, t in enumerate((a11 + a22, a21 + a22, a22, a11 + a12, a11, a21 - a11, a12 - a22)):
            for kt in range(2):
                a_ref[i, kt] = pk(t[:, kt * 128:(kt + 1) * 128].astype(bf16))
        arp = jnp.concatenate([a[:, KM:], jnp.zeros((D, 128 - KR), f32)], axis=1).astype(bf16)
        ar_ref[0] = pk(arp[:MH])
        ar_ref[1] = pk(arp[MH:])
        c_ = jnp.sum(wt * br, axis=1, keepdims=True)
        c_ref[...] = jnp.broadcast_to(c_, (D, 128))

        def tok(t):
            return [pltpu.bitcast(t[i:i + 8], u32) for i in range(0, t.shape[0], 8)]

        def stats(s, q):
            cols = slice(q * QT, (q + 1) * QT)
            k0 = xbuf[s, 0:16, cols].astype(f32)[0:1]
            acc1 = acc2 = None
            toks = []
            for c in range(D // 32):
                d = xbuf[s, 32 * c:32 * c + 32, cols].astype(f32) - k0
                dd = d * d
                for j in range(4):
                    p1, p2 = d[8 * j:8 * j + 8], dd[8 * j:8 * j + 8]
                    acc1 = p1 if acc1 is None else acc1 + p1
                    acc2 = p2 if acc2 is None else acc2 + p2
                toks.append(tok(acc1[:, :HT]) + tok(acc1[:, HT:]) + tok(acc2[:, :HT]) + tok(acc2[:, HT:]))
            s1 = jnp.sum(acc1, axis=0, keepdims=True) * (1.0 / D)
            s2 = jnp.sum(acc2, axis=0, keepdims=True) * (1.0 / D)
            m = k0 + s1
            v = jnp.maximum(s2 - s1 * s1, 0.0)
            r = jax.lax.rsqrt(v + 1e-5)
            return (m, r), toks

        def norm(s, q, slot, m, r):
            cols = slice(q * QT, (q + 1) * QT)
            cat = lambda p, q_: jnp.concatenate([p, q_], axis=1).astype(bf16)
            toks = []
            o6s = []
            for c in range(KH // 16):
                r0 = 16 * c
                top = (xbuf[s, r0:r0 + 16, cols].astype(f32) - m) * r
                bot = (xbuf[s, KH + r0:KH + r0 + 16, cols].astype(f32) - m) * r
                b11, b12, b21, b22 = top[:, :HT], top[:, HT:], bot[:, :HT], bot[:, HT:]
                o3, o4 = b12 - b22, b21 - b11
                bb_ref[slot, r0:r0 + 16] = cat(b11 + b22, b11)
                bb_ref[slot, 256 + r0:256 + r0 + 16] = cat(o4, b22)
                bb_ref[slot, 512 + r0:512 + r0 + 16] = cat(o3, b11 + b12)
                o6s.append(b21 + b22)
                if c % 2 == 1:
                    bb_ref[slot, 768 + 8 * (c - 1):768 + 8 * (c - 1) + 16] = cat(o6s[-2], o6s[-1])
                toks.append(tok(o3) + tok(o4))
            for c in range(KR // 16):
                r0 = 16 * c
                xn = (xbuf[s, KM + r0:KM + r0 + 16, cols].astype(f32) - m) * r
                bb_ref[slot, 896 + r0:896 + r0 + 16] = xn.astype(bf16)
                toks.append(tok(xn[:, :HT]) + tok(xn[:, HT:]))
            return toks

        def mm(s, q, slot, gates, fmask):
            def lhs(ref_tile, key):
                rows = []
                for j in range(NR):
                    t = ref_tile[8 * j:8 * j + 8]
                    for tk in gates.get(key + (j,), ()):
                        t = jnp.where(fmask, tk, t)
                    rows.append(t)
                return upk(jnp.concatenate(rows, axis=0))
            def prod(i, rhs):
                ai = jnp.concatenate([lhs(a_ref.at[i, 0], (i, 0)), lhs(a_ref.at[i, 1], (i, 1))], axis=1)
                return jnp.dot(ai, rhs, preferred_element_type=f32)
            def rprod(l, j):
                return jnp.dot(l, bb_ref[slot, 896:960, j * HT:(j + 1) * HT], preferred_element_type=f32)
            m1 = prod(0, bb_ref[slot, 0:256, :HT]); m2 = prod(1, bb_ref[slot, 0:256, HT:])
            c22 = m1 - m2
            m4 = prod(2, bb_ref[slot, 256:512, :HT]); m5 = prod(3, bb_ref[slot, 256:512, HT:])
            c11 = m1 + m4 - m5
            c21 = m2 + m4
            m3 = prod(4, bb_ref[slot, 512:768, :HT]); m6 = prod(5, bb_ref[slot, 512:768, HT:])
            c22 = c22 + m3 + m6
            c12 = m5 + m3
            b7 = jnp.concatenate(
                [bb_ref[slot, 768 + 16 * c:768 + 16 * c + 16, h * HT:(h + 1) * HT]
                 for c in range(8) for h in range(2)], axis=0)
            m7 = prod(6, b7)
            ct, cbm = c_ref[:MH], c_ref[MH:]
            l0 = lhs(ar_ref.at[0], (7, 0))[:, :KR]
            c11 = c11 + m7 + rprod(l0, 0) + ct
            c12 = c12 + rprod(l0, 1) + ct
            l1 = lhs(ar_ref.at[1], (8, 0))[:, :KR]
            c21 = c21 + rprod(l1, 0) + cbm
            c22 = c22 + rprod(l1, 1) + cbm
            t0 = q * QT
            obuf[s, :MH, t0:t0 + QT] = jnp.concatenate([c11, c12], axis=1).astype(bf16)
            obuf[s, MH:, t0:t0 + QT] = jnp.concatenate([c21, c22], axis=1).astype(bf16)

        def assign(u, groups):
            slots = []
            for p in range(9):
                ph = (p + (u % 2)) // 2
                for j in range(NR):
                    for kt in range(2 if p < 7 else 1):
                        slots.append((ph * NR + j - (NR // 2 if u % 2 else 0), (p, kt, j)))
            slots.sort()
            used = [False] * len(slots)
            gates = {}
            for t0, t1, tgs in groups:
                flat = [t for tg in tgs for t in tg]
                for n, t in enumerate(flat):
                    want = t0 + (t1 - t0) * n / len(flat)
                    best = None
                    for i, (tm, key) in enumerate(slots):
                        if not used[i] and tm >= want:
                            best = i
                            break
                    if best is None:
                        best = max(i for i in range(len(slots)) if not used[i])
                    used[best] = True
                    gates.setdefault(slots[best][1], []).append(t)
            return gates

        def issue_reads(s):
            for k in range(RPI):
                t = LOOK + RPI * s + k
                @pl.when(t < S)
                def _():
                    in_copy(t).start()

        def issue_writes(s):
            @pl.when(s == WSTART)
            def _():
                for t in range(WSTART):
                    out_copy(t).start()
            @pl.when(s >= WSTART)
            def _():
                out_copy(s).start()

        in_copy(0).wait()
        (m0, r0), _ = stats(0, 0)
        norm(0, 0, 0, m0, r0)
        (m1_, r1_), _ = stats(0, 1)
        st_ref[0, 0:1] = m1_
        st_ref[0, 1:2] = r1_

        def block(s0, h, fmask):
            for k in range(SB):
                issue_reads(s0 + k)
            for k in range(1, SB + 1):
                @pl.when(s0 + k < S)
                def _():
                    in_copy(s0 + k).wait()
            snext = jnp.minimum(s0 + SB, S - 1)
            units = [(s0 + k, q) for k in range(SB) for q in range(NQ)] + [(snext, 0), (snext, 1)]
            slots = [h * NU] + list(range(1, NU)) + [(1 - h) * NU]
            st = (st_ref[h, 0:1], st_ref[h, 1:2])
            for u in range(NU):
                ntoks = norm(*units[u + 1], slots[u + 1], *st)
                st, stoks = stats(*units[u + 2])
                gates = assign(u, [(NORM_T0, NORM_T1, ntoks), (STAT_T0, STAT_T1, stoks)])
                mm(*units[u], slots[u], gates, fmask)
            st_ref[1 - h, 0:1] = st[0]
            st_ref[1 - h, 1:2] = st[1]
            for k in range(SB):
                issue_writes(s0 + k)

        def body(i, carry):
            zero = jax.lax.shift_right_logical(i, 10)
            fmask = jax.lax.broadcasted_iota(jnp.int32, (8, 128), 0) < zero
            for h in range(2):
                block((2 * i + h) * SB, h, fmask)
            return carry

        jax.lax.fori_loop(0, NIT // 2, body, 0)
        for s in range(S):
            out_copy(s).wait()

    out = pl.pallas_call(
        kernel,
        in_specs=[pl.BlockSpec(memory_space=pl.ANY)] * 4,
        out_specs=pl.BlockSpec(memory_space=pl.ANY),
        out_shape=jax.ShapeDtypeStruct((S, D, B), x.dtype),
        scratch_shapes=[pltpu.VMEM((S, D, B), bf16),
                        pltpu.VMEM((S, D, B), bf16),
                        pltpu.VMEM((D, D), bf16),
                        pltpu.VMEM((D,), bf16),
                        pltpu.VMEM((D,), bf16),
                        pltpu.VMEM((7, 2, MH // 2, 128), u32),
                        pltpu.VMEM((2, MH // 2, 128), u32),
                        pltpu.VMEM((D, 128), f32),
                        pltpu.VMEM((NU + 1, 960, QT), bf16),
                        pltpu.VMEM((2, 8, QT), f32),
                        pltpu.SemaphoreType.DMA((S,)),
                        pltpu.SemaphoreType.DMA((S,)),
                        pltpu.SemaphoreType.DMA((3,))],
        compiler_params=pltpu.CompilerParams(
            vmem_limit_bytes=110 * 1024 * 1024, disable_bounds_checks=NOBC),
    )(xt, g, b, w)
    return jnp.transpose(out, (2, 0, 1))
```

```python
import jax
import jax.numpy as jnp
import jax.experimental.pallas as pl
import jax.experimental.pallas.tpu as pltpu

BU = 8
HEAD = (2, 4)
WSB = 5
INBLK = True
NOBC = True
NOSC = False
SLOW = 2
GPB = 3
NORM_T0, NORM_T1 = 0, 56
STAT_T0, STAT_T1 = 0, 76

@jax.jit
def pallas_standalone__layernorm_linear__sampling_kernel(x, g, b, w):
    B, S, D = x.shape
    xt = jnp.transpose(x, (1, 2, 0))
    f32, bf16, u32 = jnp.float32, jnp.bfloat16, jnp.uint32
    HT = 128
    QT = 2 * HT
    NQ = B // QT
    NUT = S * NQ
    KH, MH = 256, D // 2
    KM = 2 * KH
    KR = D - KM
    NR = MH // 16
    SPB = BU // NQ
    U0 = sum(HEAD)
    assert (U0 + 2) % NQ == 0 and BU % NQ == 0
    NLB = ((NUT - U0) // BU - 1) // 2 * 2
    UT = U0 + NLB * BU
    SL0 = (U0 + 2) // NQ
    NG = (S - SL0) // SPB
    assert (S - SL0) % SPB == 0
    MAXU = max(BU, NUT - UT)
    assert len(HEAD) >= 2
    started = {0, 1}
    for k in range(NLB):
        for t in range(GPB):
            j = ((k + 2 if t == 0 else NG) if k < SLOW else SLOW + 2 + GPB * (k - SLOW) + t)
            if j < NG:
                assert j not in started
                started.add(j)
        assert k in started
    assert started == set(range(NG)), started
    assert 0 <= WSB < NLB

    def pk(t):
        return pltpu.bitcast(t, u32)

    def upk(t):
        return pltpu.bitcast(t, bf16)

    def kernel(x_hbm, g_hbm, b_hbm, w_hbm, o_hbm,
               xbuf, obuf, w_ref, g_ref, b_ref, a_ref, ar_ref, c_ref, bb_ref, st_ref,
               sem_h, sem_g, sem_out, sem_p):
        def head_copy(j):
            s, c = j // 2, pl.ds(pl.multiple_of((j % 2) * 512, 512), 512)
            return pltpu.make_async_copy(x_hbm.at[s, :, c], xbuf.at[s, :, c], sem_h.at[j])

        def grp_copy(k):
            sl = pl.ds(SL0 + k * SPB, SPB)
            return pltpu.make_async_copy(x_hbm.at[sl], xbuf.at[sl], sem_g.at[k])

        def out_slices(s, n):
            return pltpu.make_async_copy(obuf.at[pl.ds(s, n)], o_hbm.at[pl.ds(s, n)], sem_out)

        def out_units(s, q, n):
            c = slice(q * QT, (q + n) * QT)
            return pltpu.make_async_copy(obuf.at[s, :, c], o_hbm.at[s, :, c], sem_out)

        cw = pltpu.make_async_copy(w_hbm, w_ref, sem_p.at[0])
        cg = pltpu.make_async_copy(g_hbm, g_ref, sem_p.at[1])
        cb = pltpu.make_async_copy(b_hbm, b_ref, sem_p.at[2])
        cg.start(); cb.start(); cw.start()

        def start_head(j, c):
            head_copy(j).start()
            return c
        jax.lax.fori_loop(0, 2 * SL0, start_head, 0)
        cw.wait(); cg.wait(); cb.wait()

        wt = w_ref[...].astype(f32).T
        gr = g_ref[...].astype(f32).reshape(1, D)
        br = b_ref[...].astype(f32).reshape(1, D)
        a = wt * gr
        a11, a12 = a[:MH, :KH], a[:MH, KH:KM]
        a21, a22 = a[MH:, :KH], a[MH:, KH:KM]
        for i, t in enumerate((a11 + a22, a21 + a22, a22, a11 + a12, a11, a21 - a11, a12 - a22)):
            for kt in range(2):
                a_ref[i, kt] = pk(t[:, kt * 128:(kt + 1) * 128].astype(bf16))
        arp = jnp.concatenate([a[:, KM:], jnp.zeros((D, 128 - KR), f32)], axis=1).astype(bf16)
        ar_ref[0] = pk(arp[:MH])
        ar_ref[1] = pk(arp[MH:])
        c_ = jnp.sum(wt * br, axis=1, keepdims=True)
        c_ref[...] = jnp.broadcast_to(c_, (D, 128))

        def tok(t):
            return [pltpu.bitcast(t[i:i + 8], u32) for i in range(0, t.shape[0], 8)]

        def stats(s, q):
            cols = slice(q * QT, (q + 1) * QT)
            k0 = xbuf[s, 0:16, cols].astype(f32)[0:1]
            acc1 = acc2 = None
            toks = []
            for c in range(D // 32):
                d = xbuf[s, 32 * c:32 * c + 32, cols].astype(f32) - k0
                dd = d * d
                for j in range(4):
                    p1, p2 = d[8 * j:8 * j + 8], dd[8 * j:8 * j + 8]
                    acc1 = p1 if acc1 is None else acc1 + p1
                    acc2 = p2 if acc2 is None else acc2 + p2
                toks.append(tok(acc1[:, :HT]) + tok(acc1[:, HT:]) + tok(acc2[:, :HT]) + tok(acc2[:, HT:]))
            s1 = jnp.sum(acc1, axis=0, keepdims=True) * (1.0 / D)
            s2 = jnp.sum(acc2, axis=0, keepdims=True) * (1.0 / D)
            m = k0 + s1
            v = jnp.maximum(s2 - s1 * s1, 0.0)
            r = jax.lax.rsqrt(v + 1e-5)
            return (m, r), toks

        def norm(s, q, slot, m, r):
            cols = slice(q * QT, (q + 1) * QT)
            cat = lambda p, q_: jnp.concatenate([p, q_], axis=1).astype(bf16)
            toks = []
            o6s = []
            for c in range(KH // 16):
                r0 = 16 * c
                top = (xbuf[s, r0:r0 + 16, cols].astype(f32) - m) * r
                bot = (xbuf[s, KH + r0:KH + r0 + 16, cols].astype(f32) - m) * r
                b11, b12, b21, b22 = top[:, :HT], top[:, HT:], bot[:, :HT], bot[:, HT:]
                o3, o4 = b12 - b22, b21 - b11
                bb_ref[slot, r0:r0 + 16] = cat(b11 + b22, b11)
                bb_ref[slot, 256 + r0:256 + r0 + 16] = cat(o4, b22)
                bb_ref[slot, 512 + r0:512 + r0 + 16] = cat(o3, b11 + b12)
                o6s.append(b21 + b22)
                if c % 2 == 1:
                    bb_ref[slot, 768 + 8 * (c - 1):768 + 8 * (c - 1) + 16] = cat(o6s[-2], o6s[-1])
                toks.append(tok(o3) + tok(o4))
            for c in range(KR // 16):
                r0 = 16 * c
                xn = (xbuf[s, KM + r0:KM + r0 + 16, cols].astype(f32) - m) * r
                bb_ref[slot, 896 + r0:896 + r0 + 16] = xn.astype(bf16)
                toks.append(tok(xn[:, :HT]) + tok(xn[:, HT:]))
            return toks

        def mm(s, q, slot, gates, fmask):
            def lhs(ref_tile, key):
                rows = []
                for j in range(NR):
                    t = ref_tile[8 * j:8 * j + 8]
                    for tk in gates.get(key + (j,), ()):
                        t = jnp.where(fmask, tk, t)
                    rows.append(t)
                return upk(jnp.concatenate(rows, axis=0))
            def prod(i, rhs):
                ai = jnp.concatenate([lhs(a_ref.at[i, 0], (i, 0)), lhs(a_ref.at[i, 1], (i, 1))], axis=1)
                return jnp.dot(ai, rhs, preferred_element_type=f32)
            def rprod(l, j):
                return jnp.dot(l, bb_ref[slot, 896:960, j * HT:(j + 1) * HT], preferred_element_type=f32)
            m1 = prod(0, bb_ref[slot, 0:256, :HT]); m2 = prod(1, bb_ref[slot, 0:256, HT:])
            c22 = m1 - m2
            m4 = prod(2, bb_ref[slot, 256:512, :HT]); m5 = prod(3, bb_ref[slot, 256:512, HT:])
            c11 = m1 + m4 - m5
            c21 = m2 + m4
            m3 = prod(4, bb_ref[slot, 512:768, :HT]); m6 = prod(5, bb_ref[slot, 512:768, HT:])
            c22 = c22 + m3 + m6
            c12 = m5 + m3
            b7 = jnp.concatenate(
                [bb_ref[slot, 768 + 16 * c:768 + 16 * c + 16, h * HT:(h + 1) * HT]
                 for c in range(8) for h in range(2)], axis=0)
            m7 = prod(6, b7)
            ct, cbm = c_ref[:MH], c_ref[MH:]
            l0 = lhs(ar_ref.at[0], (7, 0))[:, :KR]
            c11 = c11 + m7 + rprod(l0, 0) + ct
            c12 = c12 + rprod(l0, 1) + ct
            l1 = lhs(ar_ref.at[1], (8, 0))[:, :KR]
            c21 = c21 + rprod(l1, 0) + cbm
            c22 = c22 + rprod(l1, 1) + cbm
            t0 = q * QT
            obuf[s, :MH, t0:t0 + QT] = jnp.concatenate([c11, c12], axis=1).astype(bf16)
            obuf[s, MH:, t0:t0 + QT] = jnp.concatenate([c21, c22], axis=1).astype(bf16)

        def assign(u, groups):
            slots = []
            for p in range(9):
                ph = (p + (u % 2)) // 2
                for j in range(NR):
                    for kt in range(2 if p < 7 else 1):
                        slots.append((ph * NR + j - (NR // 2 if u % 2 else 0), (p, kt, j)))
            slots.sort()
            used = [False] * len(slots)
            gates = {}
            for t0, t1, tgs in groups:
                flat = [t for tg in tgs for t in tg]
                for n, t in enumerate(flat):
                    want = t0 + (t1 - t0) * n / len(flat)
                    best = None
                    for i, (tm, key) in enumerate(slots):
                        if not used[i] and tm >= want:
                            best = i
                            break
                    if best is None:
                        best = max(i for i in range(len(slots)) if not used[i])
                    used[best] = True
                    gates.setdefault(slots[best][1], []).append(t)
            return gates

        def block(sbase, u0, n, h, fmask, after_unit=None):
            loc = lambda u: (sbase + u // NQ, u % NQ)
            last = lambda u: isinstance(sbase, int) and sbase * NQ + u >= NUT
            slots = [h] + list(range(2, n + 1)) + [1 - h]
            st = (st_ref[h, 0:1], st_ref[h, 1:2])
            for j in range(n):
                u = u0 + j
                groups = []
                if not last(u + 1):
                    groups.append((NORM_T0, NORM_T1, norm(*loc(u + 1), slots[j + 1], *st)))
                if not last(u + 2):
                    st, stoks = stats(*loc(u + 2))
                    groups.append((STAT_T0, STAT_T1, stoks))
                mm(*loc(u), slots[j], assign(j, groups), fmask)
                if after_unit is not None:
                    after_unit(u)
            if not last(u0 + n + 1):
                st_ref[1 - h, 0:1] = st[0]
                st_ref[1 - h, 1:2] = st[1]

        def false_mask(zero):
            return jax.lax.broadcasted_iota(jnp.int32, (8, 128), 0) < zero

        cbits = pltpu.bitcast(c_ref[0:8], jnp.int32)
        fm0 = jnp.logical_and(cbits > 0, cbits < 0)
        head_copy(0).wait()
        (m0, r0), _ = stats(0, 0)
        norm(0, 0, 0, m0, r0)
        (m1_, r1_), _ = stats(0, 1)
        st_ref[0, 0:1] = m1_
        st_ref[0, 1:2] = r1_
        u, h, waited = 0, 0, 1
        for bi, n in enumerate(HEAD):
            if bi >= len(HEAD) - 2:
                grp_copy(bi - (len(HEAD) - 2)).start()
            need = (u + n + 1) // 2 + 1
            for j in range(waited, need):
                head_copy(j).wait()
            waited = need
            block(0, u, n, h, fm0)
            u += n
            h = 1 - h
        assert waited == 2 * SL0
        h0 = h

        def body(i, carry):
            fmask = false_mask(jax.lax.shift_right_logical(i, 10))
            for hh in range(2):
                k = 2 * i + hh
                for t in range(GPB):
                    j = jnp.where(k < SLOW, k + 2 if t == 0 else NG, SLOW + 2 + GPB * (k - SLOW) + t)
                    @pl.when(j < NG)
                    def _():
                        grp_copy(j).start()
                grp_copy(k).wait()
                sbase = k * SPB

                def after(u, k=k, sbase=sbase):
                    if u % NQ == NQ - 1:
                        @pl.when(k >= WSB)
                        def _():
                            out_slices(sbase + u // NQ, 1).start()

                @pl.when(k == WSB)
                def _():
                    out_slices(0, U0 // NQ + WSB * SPB).start()
                block(sbase, U0, BU, (h0 + hh) % 2, fmask, after if INBLK else None)
                if not INBLK:
                    @pl.when(k >= WSB)
                    def _():
                        out_slices(sbase + U0 // NQ, SPB).start()
            return carry

        jax.lax.fori_loop(0, NLB // 2, body, 0)

        for k in range(NLB, NG):
            grp_copy(k).wait()

        def after_tail(u):
            s, q = u // NQ, u % NQ
            if s == S - 1:
                out_units(s, q, 1).start()
            elif q == NQ - 1:
                out_slices(s, 1).start()

        block(0, UT, NUT - UT, h0, fm0, after_tail)
        out_slices(0, S).wait()

    out = pl.pallas_call(
        kernel,
        grid=(1,),
        in_specs=[pl.BlockSpec(memory_space=pl.ANY)] * 4,
        out_specs=pl.BlockSpec(memory_space=pl.ANY),
        out_shape=jax.ShapeDtypeStruct((S, D, B), x.dtype),
        scratch_shapes=[pltpu.VMEM((S, D, B), bf16),
                        pltpu.VMEM((S, D, B), bf16),
                        pltpu.VMEM((D, D), bf16),
                        pltpu.VMEM((D,), bf16),
                        pltpu.VMEM((D,), bf16),
                        pltpu.VMEM((7, 2, MH // 2, 128), u32),
                        pltpu.VMEM((2, MH // 2, 128), u32),
                        pltpu.VMEM((D, 128), f32),
                        pltpu.VMEM((MAXU + 1, 960, QT), bf16),
                        pltpu.VMEM((2, 8, QT), f32),
                        pltpu.SemaphoreType.DMA((2 * SL0,)),
                        pltpu.SemaphoreType.DMA((NG,)),
                        pltpu.SemaphoreType.DMA(()),
                        pltpu.SemaphoreType.DMA((3,))],
        compiler_params=pltpu.CompilerParams(
            dimension_semantics=("arbitrary",),
            vmem_limit_bytes=110 * 1024 * 1024, disable_bounds_checks=NOBC,
            disable_semaphore_checks=NOSC),
    )(xt, g, b, w)
    return jnp.transpose(out, (2, 0, 1))
```

```python
import jax
import jax.numpy as jnp
import jax.experimental.pallas as pl
import jax.experimental.pallas.tpu as pltpu

BU = 4
HEAD = (1, 1, 2)
MINTAIL = 4
WSB = 6
NOBC = True
NOSC = False
NORM_T = (0, 88)
STAT_T = (70, 150)
H_STAT = (0, 40)
H_NORM = (46, 128)
H_STAT2 = (80, 150)

@jax.jit
def pallas_standalone__layernorm_linear__sampling_kernel(x, g, b, w):
    B, S, D = x.shape
    xt = jnp.transpose(x, (1, 2, 0))
    f32, bf16, u32 = jnp.float32, jnp.bfloat16, jnp.uint32
    L = 128
    QT = 4 * L
    NQ = B // QT
    NUT = S * NQ
    MH, MQ = D // 2, D // 4
    KM = 4 * L
    KR = D - KM
    SPB = BU // NQ
    U0 = sum(HEAD)
    assert BU % NQ == 0
    NLB = ((NUT - U0 - MINTAIL) // BU) // 2 * 2
    UT = U0 + NLB * BU
    NH1 = (U0 + 2 + NQ - 1) // NQ * NQ
    SL0 = NH1 // NQ
    NG = -(-(S - SL0) // SPB)
    MAXU = max(BU, NUT - UT, max(HEAD))
    NT = 40
    BROWS = NT // 2 * L + 2 * KR
    assert 0 <= WSB < NLB
    cover = [0] * NUT
    for k in range(NLB):
        if k == WSB:
            for u in range((U0 // NQ + WSB * SPB) * NQ): cover[u] += 1
        for u in range(U0, U0 + BU):
            if u % NQ == NQ - 1 and k >= WSB:
                for q in range(NQ): cover[(k * SPB + u // NQ) * NQ + q] += 1
    if UT // NQ == S - 1 and UT % NQ:
        for q in range(UT % NQ): cover[(S - 1) * NQ + q] += 1
    for u in range(UT, NUT):
        if u // NQ == S - 1: cover[u] += 1
        elif u % NQ == NQ - 1:
            for q in range(NQ): cover[u // NQ * NQ + q] += 1
    assert cover == [1] * NUT, cover

    def grp_range(k):
        lo = SL0 + k * SPB
        return lo, min(SPB, S - lo)
    for k in range(NLB):
        assert (U0 + (k + 1) * BU + 1) // NQ < SL0 + (k + 1) * SPB
        assert grp_range(k)[1] == SPB

    def pk(t):
        return pltpu.bitcast(t, u32)

    def upk(t):
        return pltpu.bitcast(t, bf16)

    def lhs_terms(a11, a12, a21, a22):
        return (a11 + a22, a21 + a22, a22, a11 + a12, a11, a21 - a11, a12 - a22)

    def rhs_terms(b11, b12, b21, b22):
        return (b11 + b22, b11, b21 - b11, b22, b12 - b22, b11 + b12, b21 + b22)

    ANTI = (True, False, True, False)
    PORD = ((0, 1, 2, 3, 4, 5, 6), (0, 1, 2, 3, 4, 5, 6), (1, 2, 0, 3, 4, 5, 6), (1, 2, 6, 0, 3, 4, 5))

    def kernel(x_hbm, g_hbm, b_hbm, w_hbm, o_hbm,
               xbuf, obuf, w_ref, g_ref, b_ref, al_ref, as_ref, ar_ref, c_ref, bb_ref, st_ref,
               sem_h, sem_g, sem_out, sem_p):
        def head_copy(j):
            s, c = j // NQ, pl.ds(pl.multiple_of((j % NQ) * QT, QT), QT)
            return pltpu.make_async_copy(x_hbm.at[s, :, c], xbuf.at[s, :, c], sem_h.at[j])

        def grp_copy(k, n=SPB):
            sl = pl.ds(SL0 + k * SPB, n)
            return pltpu.make_async_copy(x_hbm.at[sl], xbuf.at[sl], sem_g.at[k])

        def out_slices(s, n):
            return pltpu.make_async_copy(obuf.at[pl.ds(s, n)], o_hbm.at[pl.ds(s, n)], sem_out)

        def out_part(s, c0, n):
            c = slice(c0, c0 + n)
            return pltpu.make_async_copy(obuf.at[s, :, c], o_hbm.at[s, :, c], sem_out)

        cw = pltpu.make_async_copy(w_hbm, w_ref, sem_p.at[0])
        cg = pltpu.make_async_copy(g_hbm, g_ref, sem_p.at[1])
        cb = pltpu.make_async_copy(b_hbm, b_ref, sem_p.at[2])
        cg.start(); cb.start(); cw.start()

        def start_head(j, c):
            head_copy(j).start()
            return c
        jax.lax.fori_loop(0, NH1, start_head, 0)

        def start_grp(k, c):
            grp_copy(k).start()
            return c
        nfull = (S - SL0) // SPB
        jax.lax.fori_loop(0, nfull, start_grp, 0)
        if nfull < NG:
            grp_copy(nfull, grp_range(nfull)[1]).start()
        cw.wait(); cg.wait(); cb.wait()

        wt = w_ref[...].astype(f32).T
        gr = g_ref[...].astype(f32).reshape(1, D)
        br = b_ref[...].astype(f32).reshape(1, D)
        a = wt * gr
        o = lhs_terms(a[:MH, :2 * L], a[:MH, 2 * L:KM], a[MH:, :2 * L], a[MH:, 2 * L:KM])
        for i, t in enumerate((o[0], o[5], o[6])):
            for kt in range(2):
                al_ref[i, kt] = pk(t[:, kt * L:(kt + 1) * L].astype(bf16))
        for i, t in enumerate(o[1:5]):
            for p, v in enumerate(lhs_terms(t[:MQ, :L], t[:MQ, L:], t[MQ:, :L], t[MQ:, L:])):
                as_ref[i, p] = pk(v.astype(bf16))
        arp = jnp.concatenate([a[:, KM:], jnp.zeros((D, L - KR), f32)], axis=1).astype(bf16)
        ar_ref[0] = pk(arp[:MH])
        ar_ref[1] = pk(arp[MH:])
        c_ = jnp.sum(wt * br, axis=1, keepdims=True)
        c_ref[...] = jnp.broadcast_to(c_, (D, L))

        def tok(t):
            return [pltpu.bitcast(t[:, i:i + L], u32) for i in range(0, t.shape[1], L)]

        def stats(s, q):
            cols = slice(q * QT, (q + 1) * QT)
            k0 = xbuf[s, 0:8, cols].astype(f32)[0:1]
            acc1 = acc2 = None
            toks = []
            for c in range(D // 64):
                d = xbuf[s, 64 * c:64 * c + 64, cols].astype(f32) - k0
                dd = d * d
                for j in range(8):
                    p1, p2 = d[8 * j:8 * j + 8], dd[8 * j:8 * j + 8]
                    acc1 = p1 if acc1 is None else acc1 + p1
                    acc2 = p2 if acc2 is None else acc2 + p2
                t1, t2 = tok(acc1), tok(acc2)
                toks += [t for pair in zip(t1, t2) for t in pair]
            s1 = jnp.sum(acc1, axis=0, keepdims=True) * (1.0 / D)
            s2 = jnp.sum(acc2, axis=0, keepdims=True) * (1.0 / D)
            m = k0 + s1
            v = jnp.maximum(s2 - s1 * s1, 0.0)
            r = jax.lax.rsqrt(v + 1e-5)
            return (m, r), toks

        def norm(s, q, slot, m, r):
            cols = slice(q * QT, (q + 1) * QT)
            toks = []
            for c in range(L // 8):
                r0 = 8 * c
                xq = [(xbuf[s, a * L + r0:a * L + r0 + 8, cols].astype(f32) - m) * r for a in range(4)]
                blk = lambda a, t: xq[a][:, t * L:(t + 1) * L]
                o = [[rhs_terms(blk(a, bb), blk(a, 2 + bb), blk(2 + a, bb), blk(2 + a, 2 + bb))
                      for bb in range(2)] for a in range(2)]
                tiles = [o[a][bb][0] for bb in range(2) for a in range(2)]
                for i in range(4):
                    c0, c1 = (1, 0) if ANTI[i] else (0, 1)
                    t = rhs_terms(o[0][c0][1 + i], o[0][c1][1 + i], o[1][c0][1 + i], o[1][c1][1 + i])
                    tiles += list(t)
                    if i in (1, 3):
                        toks += tok(t[2]) + tok(t[4])
                tiles += [o[a][bb][5] for bb in range(2) for a in range(2)]
                tiles += [o[a][bb][6] for bb in range(2) for a in range(2)]
                for j in (0, 1, 2, 3, 4, 9, 10, 11):
                    toks += tok(tiles[2 * j])
                for j in range(NT // 2):
                    bb_ref[slot, j * L + r0:j * L + r0 + 8] = jnp.concatenate(
                        [tiles[2 * j], tiles[2 * j + 1]], axis=1).astype(bf16)
            for c in range(KR // 8):
                r0 = 8 * c
                xn = (xbuf[s, KM + r0:KM + r0 + 8, cols].astype(f32) - m) * r
                for j in range(2):
                    o0 = NT // 2 * L + j * KR + r0
                    bb_ref[slot, o0:o0 + 8] = xn[:, 2 * j * L:(2 * j + 2) * L].astype(bf16)
                toks += tok(xn)
            return toks

        def mm(s, q, slot, gates, fmask, mid=None):
            def lhs(ref_tile, key, nr):
                rows = []
                for j in range(nr):
                    t = ref_tile[8 * j:8 * j + 8]
                    tks = gates.get((key, j), ())
                    if tks:
                        tk = tks[0]
                        for e in tks[1:]:
                            tk = tk | e
                        t = jnp.where(fmask, tk, t)
                    rows.append(t)
                return upk(jnp.concatenate(rows, axis=0))
            def tile(t):
                return bb_ref[slot, (t // 2) * L:(t // 2 + 1) * L, (t % 2) * L:(t % 2 + 1) * L]
            def rem(t):
                o0 = NT // 2 * L + (t // 2) * KR
                return bb_ref[slot, o0:o0 + KR, (t % 2) * L:(t % 2 + 1) * L]
            def dot(p, q_):
                return jnp.dot(p, q_, preferred_element_type=f32)
            def al(i, g):
                return jnp.concatenate([lhs(al_ref.at[i, kt], ('l', g, kt), 18) for kt in range(2)], axis=1)
            def rhs1(t0, bb):
                return jnp.concatenate([tile(t0 + 2 * bb), tile(t0 + 2 * bb + 1)], axis=0)
            halves = lambda r: [r[:MQ], r[MQ:]]

            a1 = al(0, 0)
            m1 = [dot(a1, rhs1(0, bb)) for bb in range(2)]
            t = {}
            g = 1
            for H, i, t0 in ((0, 2, 36), (1, 1, 32)):
                for bb in range(2):
                    st_ref[2] = jnp.zeros((8, QT), f32)
                    prod = dot(al(i, g), rhs1(t0, bb))
                    l = lhs(ar_ref.at[H], ('r', g), 18)[:, :KR]
                    cb_ = c_ref[H * MH:(H + 1) * MH]
                    t[(H, H, bb)] = halves(m1[bb] + prod + dot(l, rem(2 * H + bb)) + cb_)
                    t[(H, 1 - H, bb)] = halves(dot(l, rem(2 * (1 - H) + bb)) + cb_)
                    g += 1

            def two(i, use):
                P = {}
                terms = {(0, 0): ((0, 1), (2, 1), (3, -1), (6, 1)), (0, 1): ((3, 1), (4, 1)),
                         (1, 0): ((1, 1), (2, 1)), (1, 1): ((0, 1), (1, -1), (4, 1), (5, 1))}
                part = {k: None for k in terms}
                todo = {k: list(v) for k, v in terms.items()}
                for p in PORD[i]:
                    P[p] = dot(lhs(as_ref.at[i, p], ('s', i, p), 9), tile(4 + 7 * i + p))
                    for k in terms:
                        for (pp, sg) in list(todo[k]):
                            if pp == p:
                                todo[k].remove((pp, sg))
                                if part[k] is None:
                                    part[k] = (P[p], sg)
                                else:
                                    v, s0_ = part[k]
                                    part[k] = ((v + P[p]) if sg == s0_ else (v - P[p]), s0_)
                        if not todo[k] and part[k] is not None:
                            v, s0_ = part[k]
                            part[k] = None
                            bb = (1 - k[1]) if ANTI[i] else k[1]
                            for (H, th, sg) in use:
                                acc = t[(H, th, bb)]
                                acc[k[0]] = (acc[k[0]] + v) if sg * s0_ > 0 else (acc[k[0]] - v)

            def emit(H, th):
                blk = jnp.concatenate(
                    [jnp.concatenate(t[(H, th, bb)], axis=0) for bb in range(2)], axis=1)
                c0 = q * QT + th * 2 * L
                obuf[s, H * MH:(H + 1) * MH, c0:c0 + 2 * L] = blk.astype(bf16)

            two(0, [(1, 0, 1), (1, 1, -1)])
            two(1, [(0, 0, 1), (1, 0, 1)])
            emit(1, 0)
            two(2, [(0, 0, -1), (0, 1, 1)])
            emit(0, 0)
            if mid is not None:
                mid(0)
            two(3, [(0, 1, 1), (1, 1, 1)])
            emit(0, 1)
            emit(1, 1)
            if mid is not None:
                mid(1)

        SLOTS = []
        for j in range(18):
            for g in range(5):
                for kt in range(2):
                    SLOTS.append((18 * g + j, (('l', g, kt), j)))
                if g:
                    SLOTS.append((18 * g + j, (('r', g), j)))
        for n in range(28):
            for j in range(9):
                SLOTS.append((90 + 9 * (n // 4) + j, (('s', n // 7, PORD[n // 7][n % 7]), j)))
        SLOTS.sort()

        def assign(groups):
            cnt = [0] * len(SLOTS)
            gates = {}
            for (t0, t1), toks in groups:
                for n, t in enumerate(toks):
                    want = int(t0 + (t1 - t0) * n / len(toks))
                    cand = [i for i, (tm, _) in enumerate(SLOTS) if tm == want]
                    best = min(cand, key=lambda i: cnt[i])
                    cnt[best] += 1
                    gates.setdefault(SLOTS[best][1], []).append(t)
            return gates

        def block(sbase, u0, n, h, fmask, after_unit=None, mid=None, lag=0):
            loc = lambda u: (sbase + u // NQ, u % NQ)
            last = lambda u: isinstance(sbase, int) and sbase * NQ + u >= NUT
            slots = [h] + list(range(2, n + 1)) + [1 - h]
            st = None if lag else (st_ref[h, 0:1], st_ref[h, 1:2])
            for j in range(n):
                u = u0 + j
                groups = []
                if j < lag:
                    st, stoks = stats(*loc(u + 1))
                    groups.append((H_STAT, stoks))
                    groups.append((H_NORM, norm(*loc(u + 1), slots[j + 1], *st)))
                    if j == lag - 1 and lag <= n:
                        st, stoks = stats(*loc(u + 2))
                        groups.append((H_STAT2, stoks))
                else:
                    if not last(u + 1):
                        groups.append((NORM_T, norm(*loc(u + 1), slots[j + 1], *st)))
                    if not last(u + 2):
                        st, stoks = stats(*loc(u + 2))
                        groups.append((STAT_T, stoks))
                mm(*loc(u), slots[j], assign(groups), fmask, (lambda hh, u=u: mid(u, hh)) if mid else None)
                if after_unit is not None:
                    after_unit(u)
            if not last(u0 + n + 1) and lag <= n:
                st_ref[1 - h, 0:1] = st[0]
                st_ref[1 - h, 1:2] = st[1]

        cbits = pltpu.bitcast(c_ref[0:8], jnp.int32)
        fm0 = jnp.logical_and(cbits > 0, cbits < 0)
        head_copy(0).wait()
        (m0, r0), _ = stats(0, 0)
        norm(0, 0, 0, m0, r0)
        assert HEAD[:2] == (1, 1)
        u, h, waited = 0, 0, 1
        for bi, n in enumerate(HEAD):
            need = 2 if bi == 0 else u + n + 2
            for j in range(waited, need):
                head_copy(j).wait()
            waited = need
            block(0, u, n, h, fm0, lag=(2, 1, 0, 0)[bi])
            u += n
            h = 1 - h
        for j in range(waited, NH1):
            head_copy(j).wait()
        h0 = h

        def body(i, carry):
            fmask = jax.lax.broadcasted_iota(jnp.int32, (8, L), 0) < jax.lax.shift_right_logical(i, 10)
            for hh in range(2):
                k = 2 * i + hh
                grp_copy(k).wait()
                sbase = k * SPB

                def after(u, k=k, sbase=sbase):
                    if u % NQ == NQ - 1:
                        @pl.when(k >= WSB)
                        def _():
                            out_slices(sbase + u // NQ, 1).start()

                @pl.when(k == WSB)
                def _():
                    out_slices(0, U0 // NQ + WSB * SPB).start()
                block(sbase, U0, BU, (h0 + hh) % 2, fmask, after)
            return carry

        jax.lax.fori_loop(0, NLB // 2, body, 0)

        for k in range(NLB, NG):
            grp_copy(k, grp_range(k)[1]).wait()

        def after_tail(u):
            s, q = u // NQ, u % NQ
            if s < S - 1 and q == NQ - 1:
                out_slices(s, 1).start()

        def mid_tail(u, hh):
            s, q = u // NQ, u % NQ
            if s == S - 1:
                out_part(s, q * QT + hh * 2 * L, 2 * L).start()

        if UT // NQ == S - 1 and UT % NQ:
            out_part(S - 1, 0, QT).start()
        block(0, UT, NUT - UT, h0, fm0, after_tail, mid_tail)
        out_slices(0, S).wait()

    out = pl.pallas_call(
        kernel,
        grid=(1,),
        in_specs=[pl.BlockSpec(memory_space=pl.ANY)] * 4,
        out_specs=pl.BlockSpec(memory_space=pl.ANY),
        out_shape=jax.ShapeDtypeStruct((S, D, B), x.dtype),
        scratch_shapes=[pltpu.VMEM((S, D, B), bf16),
                        pltpu.VMEM((S, D, B), bf16),
                        pltpu.VMEM((D, D), bf16),
                        pltpu.VMEM((D,), bf16),
                        pltpu.VMEM((D,), bf16),
                        pltpu.VMEM((3, 2, MH // 2, L), u32),
                        pltpu.VMEM((4, 7, MQ // 2, L), u32),
                        pltpu.VMEM((2, MH // 2, L), u32),
                        pltpu.VMEM((D, L), f32),
                        pltpu.VMEM((MAXU + 1, BROWS, 2 * L), bf16),
                        pltpu.VMEM((3, 8, QT), f32),
                        pltpu.SemaphoreType.DMA((NH1,)),
                        pltpu.SemaphoreType.DMA((NG,)),
                        pltpu.SemaphoreType.DMA(()),
                        pltpu.SemaphoreType.DMA((3,))],
        compiler_params=pltpu.CompilerParams(
            dimension_semantics=("arbitrary",),
            vmem_limit_bytes=110 * 1024 * 1024, disable_bounds_checks=NOBC,
            disable_semaphore_checks=NOSC),
    )(xt, g, b, w)
    return jnp.transpose(out, (2, 0, 1))
```

```python
import jax
import jax.numpy as jnp
import jax.experimental.pallas as pl
import jax.experimental.pallas.tpu as pltpu

BUS = (4, 8)
HEAD = (1, 1, 2)
WSB = 4
NOBC = True
NOSC = True
NORM_T = (20, 90)
STAT_T = (2, 100)
H_STAT = (2, 40)
H_NORM = (46, 128)
H_STAT2 = (80, 150)

@jax.jit
def pallas_standalone__layernorm_linear__sampling_kernel(x, g, b, w):
    B, S, D = x.shape
    xt = jnp.transpose(x, (1, 2, 0))
    f32, bf16, u32 = jnp.float32, jnp.bfloat16, jnp.uint32
    L = 128
    QT = 4 * L
    NQ = B // QT
    NUT = S * NQ
    MH, MQ = D // 2, D // 4
    KM = 4 * L
    KR = D - KM
    U0 = sum(HEAD)
    UI = sum(BUS)
    SI = UI // NQ
    NIT = (NUT - U0) // UI
    assert U0 % NQ == 0 and all(n % NQ == 0 for n in BUS) and U0 + NIT * UI == NUT
    NH1 = U0 + 2
    SL0 = NH1 // NQ
    BOFF = (U0, U0 + BUS[0])
    GLO = (SL0, SL0 + BUS[0] // NQ)
    GN = (BUS[0] // NQ, BUS[1] // NQ)
    MAXU = max(max(BUS), max(HEAD))
    NT = 40
    BROWS = NT // 2 * L + 2 * KR
    have = set(range(SL0))
    cover = [0] * (2 * NUT)
    for i in range(NIT):
        for hh in range(2):
            k = 2 * i + hh
            lo = GLO[hh] + i * SI
            grp = [s for s in range(lo, lo + GN[hh]) if s < S]
            assert len(grp) == GN[hh] - (1 if (i == NIT - 1 and hh == 1) else 0)
            assert not (have & set(grp))
            have |= set(grp)
            u0 = i * UI + BOFF[hh]
            assert all(min(u, NUT - 1) // NQ in have for u in range(u0, u0 + BUS[hh] + 2))
            if k == WSB:
                for j in range(2 * u0): cover[j] += 1
            for u in range(u0, u0 + BUS[hh]):
                if u // NQ == S - 1:
                    cover[2 * u] += 1; cover[2 * u + 1] += 1
                elif k >= WSB:
                    cover[2 * u] += 1; cover[2 * u + 1] += 1
    assert have == set(range(S)) and cover == [1] * (2 * NUT) and 0 <= WSB < 2 * NIT

    def pk(t):
        return pltpu.bitcast(t, u32)

    def upk(t):
        return pltpu.bitcast(t, bf16)

    def lhs_terms(a11, a12, a21, a22):
        return (a11 + a22, a21 + a22, a22, a11 + a12, a11, a21 - a11, a12 - a22)

    def rhs_terms(b11, b12, b21, b22):
        return (b11 + b22, b11, b21 - b11, b22, b12 - b22, b11 + b12, b21 + b22)

    ANTI = (True, False, True, False)
    PORD = ((0, 1, 2, 3, 4, 5, 6), (0, 1, 2, 3, 4, 5, 6), (1, 2, 0, 3, 4, 5, 6), (1, 2, 6, 0, 3, 4, 5))

    def kernel(x_hbm, g_hbm, b_hbm, w_hbm, o_hbm,
               xbuf, obuf, w_ref, g_ref, b_ref, al_ref, as_ref, ar_ref, c_ref, bb_ref, st_ref,
               sem_h, sem_g, sem_out, sem_p):
        def head_copy(j):
            s, c = j // NQ, pl.ds(pl.multiple_of((j % NQ) * QT, QT), QT)
            return pltpu.make_async_copy(x_hbm.at[s, :, c], xbuf.at[s, :, c], sem_h.at[j])

        def grp_copy(i, hh, short=False):
            sl = pl.ds(GLO[hh] + i * SI, GN[hh] - (1 if short else 0))
            return pltpu.make_async_copy(x_hbm.at[sl], xbuf.at[sl], sem_g.at[2 * i + hh])

        def out_slices(s, n):
            return pltpu.make_async_copy(obuf.at[pl.ds(s, n)], o_hbm.at[pl.ds(s, n)], sem_out)

        def out_part(s, rows, c0, n):
            c = slice(c0, c0 + n)
            return pltpu.make_async_copy(obuf.at[s, rows, c], o_hbm.at[s, rows, c], sem_out)

        cw = pltpu.make_async_copy(w_hbm, w_ref, sem_p.at[0])
        cg = pltpu.make_async_copy(g_hbm, g_ref, sem_p.at[1])
        cb = pltpu.make_async_copy(b_hbm, b_ref, sem_p.at[2])
        cg.start(); cb.start(); cw.start()

        def start_head(j, c):
            head_copy(j).start()
            return c
        jax.lax.fori_loop(0, NH1, start_head, 0)

        def start_grp(k, c):
            i = k // 2
            pl.when(k % 2 == 0)(lambda: grp_copy(i, 0).start())
            pl.when(jnp.logical_and(k % 2 == 1, i < NIT - 1))(lambda: grp_copy(i, 1).start())
            pl.when(k == 2 * NIT - 1)(lambda: grp_copy(i, 1, True).start())
            return c
        jax.lax.fori_loop(0, 2 * NIT, start_grp, 0)
        cw.wait(); cg.wait(); cb.wait()

        wt = w_ref[...].astype(f32).T
        gr = g_ref[...].astype(f32).reshape(1, D)
        br = b_ref[...].astype(f32).reshape(1, D)
        a = wt * gr
        o = lhs_terms(a[:MH, :2 * L], a[:MH, 2 * L:KM], a[MH:, :2 * L], a[MH:, 2 * L:KM])
        for i, t in enumerate((o[0], o[5], o[6])):
            for kt in range(2):
                al_ref[i, kt] = pk(t[:, kt * L:(kt + 1) * L].astype(bf16))
        for i, t in enumerate(o[1:5]):
            for p, v in enumerate(lhs_terms(t[:MQ, :L], t[:MQ, L:], t[MQ:, :L], t[MQ:, L:])):
                as_ref[i, p] = pk(v.astype(bf16))
        arp = jnp.concatenate([a[:, KM:], jnp.zeros((D, L - KR), f32)], axis=1).astype(bf16)
        ar_ref[0] = pk(arp[:MH])
        ar_ref[1] = pk(arp[MH:])
        c_ = jnp.sum(wt * br, axis=1, keepdims=True)
        c_ref[...] = jnp.broadcast_to(c_, (D, L))

        def tok(t):
            return [pltpu.bitcast(t[:, i:i + L], u32) for i in range(0, t.shape[1], L)]

        def stats(s, q):
            cols = slice(q * QT, (q + 1) * QT)
            k0 = xbuf[s, 0:8, cols].astype(f32)[0:1]
            acc1 = acc2 = None
            toks = []
            for c in range(D // 64):
                d = xbuf[s, 64 * c:64 * c + 64, cols].astype(f32) - k0
                dd = d * d
                for j in range(8):
                    p1, p2 = d[8 * j:8 * j + 8], dd[8 * j:8 * j + 8]
                    acc1 = p1 if acc1 is None else acc1 + p1
                    acc2 = p2 if acc2 is None else acc2 + p2
                t1, t2 = tok(acc1), tok(acc2)
                toks += [t for pair in zip(t1, t2) for t in pair]
            s1 = jnp.sum(acc1, axis=0, keepdims=True) * (1.0 / D)
            s2 = jnp.sum(acc2, axis=0, keepdims=True) * (1.0 / D)
            m = k0 + s1
            v = jnp.maximum(s2 - s1 * s1, 0.0)
            r = jax.lax.rsqrt(v + 1e-5)
            return (m, r), toks

        def norm(s, q, slot, m, r):
            cols = slice(q * QT, (q + 1) * QT)
            toks = []
            for c in range(L // 8):
                r0 = 8 * c
                xq = [(xbuf[s, a * L + r0:a * L + r0 + 8, cols].astype(f32) - m) * r for a in range(4)]
                blk = lambda a, t: xq[a][:, t * L:(t + 1) * L]
                o = [[rhs_terms(blk(a, bb), blk(a, 2 + bb), blk(2 + a, bb), blk(2 + a, 2 + bb))
                      for bb in range(2)] for a in range(2)]
                tiles = [o[a][bb][0] for bb in range(2) for a in range(2)]
                for i in range(4):
                    c0, c1 = (1, 0) if ANTI[i] else (0, 1)
                    t = rhs_terms(o[0][c0][1 + i], o[0][c1][1 + i], o[1][c0][1 + i], o[1][c1][1 + i])
                    tiles += list(t)
                    if i in (1, 3):
                        toks += tok(t[2]) + tok(t[4])
                tiles += [o[a][bb][5] for bb in range(2) for a in range(2)]
                tiles += [o[a][bb][6] for bb in range(2) for a in range(2)]
                for j in (0, 1, 2, 3, 4, 9, 10, 11):
                    toks += tok(tiles[2 * j])
                for j in range(NT // 2):
                    bb_ref[slot, j * L + r0:j * L + r0 + 8] = jnp.concatenate(
                        [tiles[2 * j], tiles[2 * j + 1]], axis=1).astype(bf16)
            for c in range(KR // 8):
                r0 = 8 * c
                xn = (xbuf[s, KM + r0:KM + r0 + 8, cols].astype(f32) - m) * r
                for j in range(2):
                    o0 = NT // 2 * L + j * KR + r0
                    bb_ref[slot, o0:o0 + 8] = xn[:, 2 * j * L:(2 * j + 2) * L].astype(bf16)
                toks += tok(xn)
            return toks

        def mm(s, q, slot, gates, fmask, mid=None):
            def lhs(ref_tile, key, nr):
                rows = []
                for j in range(nr):
                    t = ref_tile[8 * j:8 * j + 8]
                    tks = gates.get((key, j), ())
                    if tks:
                        tk = tks[0]
                        for e in tks[1:]:
                            tk = tk | e
                        t = jnp.where(fmask, tk, t)
                    rows.append(t)
                return upk(jnp.concatenate(rows, axis=0))
            def tile(t):
                return bb_ref[slot, (t // 2) * L:(t // 2 + 1) * L, (t % 2) * L:(t % 2 + 1) * L]
            def rem(t):
                o0 = NT // 2 * L + (t // 2) * KR
                return bb_ref[slot, o0:o0 + KR, (t % 2) * L:(t % 2 + 1) * L]
            def dot(p, q_):
                return jnp.dot(p, q_, preferred_element_type=f32)
            def al(i, g):
                return jnp.concatenate([lhs(al_ref.at[i, kt], ('l', g, kt), 18) for kt in range(2)], axis=1)
            def rhs1(t0, bb):
                return jnp.concatenate([tile(t0 + 2 * bb), tile(t0 + 2 * bb + 1)], axis=0)
            halves = lambda r: [r[:MQ], r[MQ:]]

            a1 = al(0, 0)
            m1 = [dot(a1, rhs1(0, bb)) for bb in range(2)]
            t = {}
            g = 1
            for H, i, t0 in ((0, 2, 36), (1, 1, 32)):
                for bb in range(2):
                    st_ref[2] = jnp.zeros((8, QT), f32)
                    prod = dot(al(i, g), rhs1(t0, bb))
                    l = lhs(ar_ref.at[H], ('r', g), 18)[:, :KR]
                    cb_ = c_ref[H * MH:(H + 1) * MH]
                    t[(H, H, bb)] = halves(m1[bb] + prod + dot(l, rem(2 * H + bb)) + cb_)
                    t[(H, 1 - H, bb)] = halves(dot(l, rem(2 * (1 - H) + bb)) + cb_)
                    g += 1

            def two(i, use):
                P = {}
                terms = {(0, 0): ((0, 1), (2, 1), (3, -1), (6, 1)), (0, 1): ((3, 1), (4, 1)),
                         (1, 0): ((1, 1), (2, 1)), (1, 1): ((0, 1), (1, -1), (4, 1), (5, 1))}
                part = {k: None for k in terms}
                todo = {k: list(v) for k, v in terms.items()}
                for p in PORD[i]:
                    P[p] = dot(lhs(as_ref.at[i, p], ('s', i, p), 9), tile(4 + 7 * i + p))
                    for k in terms:
                        for (pp, sg) in list(todo[k]):
                            if pp == p:
                                todo[k].remove((pp, sg))
                                if part[k] is None:
                                    part[k] = (P[p], sg)
                                else:
                                    v, s0_ = part[k]
                                    part[k] = ((v + P[p]) if sg == s0_ else (v - P[p]), s0_)
                        if not todo[k] and part[k] is not None:
                            v, s0_ = part[k]
                            part[k] = None
                            bb = (1 - k[1]) if ANTI[i] else k[1]
                            for (H, th, sg) in use:
                                acc = t[(H, th, bb)]
                                acc[k[0]] = (acc[k[0]] + v) if sg * s0_ > 0 else (acc[k[0]] - v)

            def emit(H, th):
                blk = jnp.concatenate(
                    [jnp.concatenate(t[(H, th, bb)], axis=0) for bb in range(2)], axis=1)
                c0 = q * QT + th * 2 * L
                obuf[s, H * MH:(H + 1) * MH, c0:c0 + 2 * L] = blk.astype(bf16)

            two(0, [(1, 0, 1), (1, 1, -1)])
            two(1, [(0, 0, 1), (1, 0, 1)])
            emit(1, 0)
            if mid is not None:
                mid(slice(MH, D), 0)
            two(2, [(0, 0, -1), (0, 1, 1)])
            emit(0, 0)
            if mid is not None:
                mid(slice(0, MH), 0)
            two(3, [(0, 1, 1), (1, 1, 1)])
            emit(0, 1)
            emit(1, 1)
            if mid is not None:
                mid(slice(0, D), 1)

        SLOTS = []
        for j in range(18):
            for g in range(5):
                for kt in range(2):
                    SLOTS.append((18 * g + j, (('l', g, kt), j)))
                if g:
                    SLOTS.append((18 * g + j, (('r', g), j)))
        for n in range(28):
            for j in range(9):
                SLOTS.append((90 + 9 * (n // 4) + j, (('s', n // 7, PORD[n // 7][n % 7]), j)))
        SLOTS.sort()

        def assign(groups):
            cnt = [0] * len(SLOTS)
            gates = {}
            for (t0, t1), toks in groups:
                for n, t in enumerate(toks):
                    want = int(t0 + (t1 - t0) * n / len(toks))
                    cand = [i for i, (tm, _) in enumerate(SLOTS) if tm == want]
                    best = min(cand, key=lambda i: cnt[i])
                    cnt[best] += 1
                    gates.setdefault(SLOTS[best][1], []).append(t)
            return gates

        def block(sbase, u0, n, h, fmask, after_unit=None, mid=None, lag=0):
            def loc(u):
                s = sbase + u // NQ
                if u >= u0 + n and not isinstance(sbase, int):
                    s = jnp.minimum(s, S - 1)
                return s, u % NQ
            last = lambda u: False
            slots = [h] + list(range(2, n + 1)) + [1 - h]
            st = None if lag else (st_ref[h, 0:1], st_ref[h, 1:2])
            for j in range(n):
                u = u0 + j
                groups = []
                if j < lag:
                    st, stoks = stats(*loc(u + 1))
                    groups.append((H_STAT, stoks))
                    groups.append((H_NORM, norm(*loc(u + 1), slots[j + 1], *st)))
                    if j == lag - 1 and lag <= n:
                        st, stoks = stats(*loc(u + 2))
                        groups.append((H_STAT2, stoks))
                else:
                    if not last(u + 1):
                        groups.append((NORM_T, norm(*loc(u + 1), slots[j + 1], *st)))
                    if not last(u + 2):
                        st, stoks = stats(*loc(u + 2))
                        groups.append((STAT_T, stoks))
                mm(*loc(u), slots[j], assign(groups), fmask, (lambda rows, th, u=u: mid(u, rows, th)) if mid else None)
                if after_unit is not None:
                    after_unit(u)
            if not last(u0 + n + 1) and lag <= n:
                st_ref[1 - h, 0:1] = st[0]
                st_ref[1 - h, 1:2] = st[1]

        cbits = pltpu.bitcast(c_ref[0:8], jnp.int32)
        fm0 = jnp.logical_and(cbits > 0, cbits < 0)
        head_copy(0).wait()
        (m0, r0), _ = stats(0, 0)
        norm(0, 0, 0, m0, r0)
        assert HEAD[:2] == (1, 1)
        u, h, waited = 0, 0, 1
        for bi, n in enumerate(HEAD):
            need = 2 if bi == 0 else u + n + 2
            for j in range(waited, need):
                head_copy(j).wait()
            waited = need
            block(0, u, n, h, fm0, lag=(2, 1, 0, 0)[bi])
            u += n
            h = 1 - h
        for j in range(waited, NH1):
            head_copy(j).wait()
        h0 = h

        def body(i, carry):
            fmask = jax.lax.broadcasted_iota(jnp.int32, (8, L), 0) < jax.lax.shift_right_logical(i, 10)
            sbase = i * SI
            for hh in range(2):
                k = 2 * i + hh
                if hh == 0:
                    grp_copy(i, 0).wait()
                else:
                    pl.when(i < NIT - 1)(lambda: grp_copy(i, 1).wait())
                    pl.when(i == NIT - 1)(lambda: grp_copy(i, 1, True).wait())
                uend = U0 + UI

                def after(u, k=k):
                    cond = k >= WSB
                    if u >= uend - NQ:
                        cond = jnp.logical_and(cond, i < NIT - 1)
                    pl.when(cond)(
                        lambda: out_part(sbase + u // NQ, slice(0, D), (u % NQ) * QT, QT).start())

                def mid(u, rows, th):
                    if u >= uend - NQ:
                        pl.when(i == NIT - 1)(
                            lambda: out_part(S - 1, rows, (u % NQ) * QT + th * 2 * L, 2 * L).start())

                if WSB % 2 == hh:
                    pl.when(k == WSB)(
                        lambda: out_slices(0, ((WSB // 2) * UI + BOFF[hh]) // NQ).start())
                block(sbase, BOFF[hh], BUS[hh], (h0 + hh) % 2, fmask, after, mid)
            return carry

        jax.lax.fori_loop(0, NIT, body, 0)
        out_slices(0, S).wait()

    out = pl.pallas_call(
        kernel,
        grid=(1,),
        in_specs=[pl.BlockSpec(memory_space=pl.ANY)] * 4,
        out_specs=pl.BlockSpec(memory_space=pl.ANY),
        out_shape=jax.ShapeDtypeStruct((S, D, B), x.dtype),
        scratch_shapes=[pltpu.VMEM((S, D, B), bf16),
                        pltpu.VMEM((S, D, B), bf16),
                        pltpu.VMEM((D, D), bf16),
                        pltpu.VMEM((D,), bf16),
                        pltpu.VMEM((D,), bf16),
                        pltpu.VMEM((3, 2, MH // 2, L), u32),
                        pltpu.VMEM((4, 7, MQ // 2, L), u32),
                        pltpu.VMEM((2, MH // 2, L), u32),
                        pltpu.VMEM((D, L), f32),
                        pltpu.VMEM((MAXU + 1, BROWS, 2 * L), bf16),
                        pltpu.VMEM((3, 8, QT), f32),
                        pltpu.SemaphoreType.DMA((NH1,)),
                        pltpu.SemaphoreType.DMA((2 * NIT,)),
                        pltpu.SemaphoreType.DMA(()),
                        pltpu.SemaphoreType.DMA((3,))],
        compiler_params=pltpu.CompilerParams(
            dimension_semantics=("arbitrary",),
            vmem_limit_bytes=110 * 1024 * 1024, disable_bounds_checks=NOBC,
            disable_semaphore_checks=NOSC),
    )(xt, g, b, w)
    return jnp.transpose(out, (2, 0, 1))
```

```python
import jax
import jax.numpy as jnp
import jax.experimental.pallas as pl
import jax.experimental.pallas.tpu as pltpu

HEAD = (1, 1, 2)
BUS = (4, 8)
WSB = 4
NORM_T, STAT_T = (18, 90), (2, 100)
HEAD_STAT_T, HEAD_NORM_T, HEAD_STAT2_T = (2, 40), (46, 120), (76, 150)
EPS = 1e-5


def _lhs_terms(a11, a12, a21, a22):
    return (a11 + a22, a21 + a22, a22, a11 + a12, a11, a11 - a21, a12 - a22)


def _rhs_terms(b11, b12, b21, b22):
    return (b11 - b22, b11, b21 - b11, b22, b12 - b22, b11 - b12, b21 - b22)


_COMB = {(0, 0): ((0, 1), (2, 1), (3, 1), (6, 1)), (0, 1): ((3, 1), (4, 1)),
         (1, 0): ((1, 1), (2, 1)), (1, 1): ((0, -1), (1, 1), (4, 1), (5, 1))}
_SWAP = (True, False, True, False)
_PORD = ((0, 1, 2, 3, 4, 5, 6), (0, 1, 2, 3, 4, 5, 6), (1, 2, 0, 3, 4, 5, 6), (1, 2, 6, 0, 3, 4, 5))


def _lane(k, t0, t1, n=72):
    rows = [(('l', grp, k), j) for grp in range(5) for j in range(18)]
    rows += [(('s', m // 7, _PORD[m // 7][m % 7]), j) for m in range(k, 28, 4) for j in range(9)]
    assert t1 - t0 >= n
    return [rows[t0 + (t1 - t0) * i // n] for i in range(n)]


@jax.jit
def pallas_standalone__layernorm_linear__sampling_kernel(x, g, b, w):
    B, S, D = x.shape
    f32, bf16 = jnp.float32, jnp.bfloat16
    L = 128
    QT = 4 * L
    NQ = B // QT
    NUT = S * NQ
    MH, MQ = D // 2, D // 4
    KM = 4 * L
    KR = D - KM
    NT = 40
    RO = NT // 2 * L
    U0, UI = sum(HEAD), sum(BUS)
    SI = UI // NQ
    NIT = (NUT - U0) // UI
    NH = U0 + 2
    SL0 = NH // NQ
    BOFF = (U0, U0 + BUS[0])
    GLO = (SL0, SL0 + BUS[0] // NQ)
    GN = (BUS[0] // NQ, BUS[1] // NQ)
    assert (B, D) == (NQ * QT, 576) and HEAD[:2] == (1, 1)
    assert U0 % NQ == 0 and all(n % NQ == 0 for n in BUS) and U0 + NIT * UI == NUT
    have, cover = set(range(SL0)), [0] * NUT
    for i in range(NIT):
        for hh in range(2):
            grp = set(range(GLO[hh] + i * SI, min(GLO[hh] + i * SI + GN[hh], S)))
            assert len(grp) == GN[hh] - (i == NIT - 1 and hh == 1) and not (have & grp)
            have |= grp
            u0 = i * UI + BOFF[hh]
            assert all(min(u, NUT - 1) // NQ in have for u in range(u0, u0 + BUS[hh] + 2))
            for u in range(u0 if 2 * i + hh != WSB else 0, u0 + BUS[hh]):
                cover[u] += 2 * i + hh >= WSB
    assert have == set(range(S)) and cover == [1] * NUT

    norm_at, stat_at = _lane(0, *NORM_T), _lane(1, *STAT_T)
    stat_h = [e for p in zip(_lane(0, *HEAD_STAT_T, 36), _lane(1, *HEAD_STAT_T, 36)) for e in p]
    norm_h, stat_h2 = _lane(0, *HEAD_NORM_T), _lane(1, *HEAD_STAT2_T)

    def kernel(x_hbm, g_hbm, b_hbm, w_hbm, o_hbm,
               xbuf, obuf, w_ref, g_ref, b_ref, al_ref, as_ref, ar_ref, c_ref, bb_ref, st_ref,
               sem_h, sem_g, sem_o, sem_p):
        def head_copy(j):
            s, c = j // NQ, pl.ds(pl.multiple_of((j % NQ) * QT, QT), QT)
            return pltpu.make_async_copy(x_hbm.at[s, :, c], xbuf.at[s, :, c], sem_h.at[j])

        def grp_copy(i, hh, short=False):
            sl = pl.ds(GLO[hh] + i * SI, GN[hh] - short)
            return pltpu.make_async_copy(x_hbm.at[sl], xbuf.at[sl], sem_g.at[2 * i + hh])

        def out_slices(s, n):
            return pltpu.make_async_copy(obuf.at[pl.ds(s, n)], o_hbm.at[pl.ds(s, n)], sem_o)

        def out_part(s, rows, c0, n):
            c = slice(c0, c0 + n)
            return pltpu.make_async_copy(obuf.at[s, rows, c], o_hbm.at[s, rows, c], sem_o)

        params = [pltpu.make_async_copy(src, dst, sem_p.at[i])
                  for i, (src, dst) in enumerate(((g_hbm, g_ref), (b_hbm, b_ref), (w_hbm, w_ref)))]
        for p in params:
            p.start()

        @pl.loop(0, NH)
        def _(j):
            head_copy(j).start()

        @pl.loop(0, 2 * NIT)
        def _(k):
            i = k // 2
            pl.when(k % 2 == 0)(lambda: grp_copy(i, 0).start())
            pl.when(jnp.logical_and(k % 2 == 1, i < NIT - 1))(lambda: grp_copy(i, 1).start())
            pl.when(k == 2 * NIT - 1)(lambda: grp_copy(i, 1, True).start())

        for p in params:
            p.wait()

        def pack(t):
            return pltpu.bitcast(t.astype(bf16), f32)

        gr = g_ref[...].astype(f32).reshape(1, D)
        wb = w_ref[...]
        mu = jnp.sum(wb.astype(f32), axis=0, keepdims=True) * (
            jnp.sum(gr, axis=1, keepdims=True) * (1.0 / (D * D)))
        wt = jnp.concatenate([wb, jnp.broadcast_to(mu.astype(bf16), (KR + L, D))], axis=0).T.astype(f32)
        mu = wt[:, D + KR:]
        wt = wt[:, :D]
        a = wt * gr - jnp.concatenate([mu] * 4 + [mu[:, :KR]], axis=1)
        o = _lhs_terms(a[:MH, :2 * L], a[:MH, 2 * L:KM], a[MH:, :2 * L], a[MH:, 2 * L:KM])
        for i, t in enumerate((o[0], o[6], o[5])):
            t = pack(t)
            for kt in range(2):
                al_ref[i, kt] = t[:, kt * L:(kt + 1) * L]
        short = [v for t in o[1:5] for v in _lhs_terms(t[:MQ, :L], t[:MQ, L:], t[MQ:, :L], t[MQ:, L:])]
        for n in range(0, 28, 2):
            t = pack(jnp.concatenate(short[n:n + 2], axis=1))
            for e in range(2):
                as_ref[(n + e) // 7, (n + e) % 7] = t[:, e * L:(e + 1) * L]
        ar = jnp.concatenate([a[:, KM:], jnp.zeros((D, L - KR), f32)], axis=1)
        t = pack(jnp.concatenate([ar[:MH], ar[MH:]], axis=1))
        for h in range(2):
            ar_ref[h] = t[:, h * L:(h + 1) * L]
        c_ref[...] = jnp.broadcast_to(
            jnp.sum(wt * b_ref[...].astype(f32).reshape(1, D), axis=1, keepdims=True), (D, L))

        def load(s, q, r0, n):
            return xbuf[s, r0:r0 + n, q * QT:(q + 1) * QT].astype(f32)

        def stats(s, q, rows=D):
            k0 = load(s, q, 0, 8)[0:1]
            acc1 = acc2 = None
            marks = []
            for r0 in range(0, D, rows):
                d = load(s, q, r0, rows) - k0
                p1 = jnp.sum(d.reshape(rows // 32, 4, 8, QT), axis=1)
                p2 = jnp.sum((d * d).reshape(rows // 32, 4, 8, QT), axis=1)
                for c in range(rows // 32):
                    acc1, acc2 = (p1[c], p2[c]) if acc1 is None else (acc1 + p1[c], acc2 + p2[c])
                    t = acc1 + acc2
                    marks += [t[:, j * L:(j + 1) * L] for j in range(4)]
            s1 = jnp.sum(acc1, axis=0, keepdims=True) * (1.0 / D)
            s2 = jnp.sum(acc2, axis=0, keepdims=True) * (1.0 / D)
            var = jnp.maximum(s2 - s1 * s1, 0.0)
            return (k0 + s1, jax.lax.rsqrt(var + EPS)), marks

        def norm(s, q, slot, mean, rstd, rows=L):
            marks = []
            for r0 in range(0, L, rows):
                xn = [(load(s, q, r * L + r0, rows) - mean) * rstd for r in range(4)]
                blk = lambda r, t: xn[r][:, t * L:(t + 1) * L]
                o = [[_rhs_terms(blk(i, j), blk(i, 2 + j), blk(2 + i, j), blk(2 + i, 2 + j))
                      for j in range(2)] for i in range(2)]
                tiles = [o[i][j][0] for j in range(2) for i in range(2)]
                for i in range(4):
                    c0, c1 = (1, 0) if _SWAP[i] else (0, 1)
                    tiles += _rhs_terms(o[0][c0][1 + i], o[0][c1][1 + i], o[1][c0][1 + i], o[1][c1][1 + i])
                tiles += [o[i][j][k] for k in (6, 5) for j in range(2) for i in range(2)]
                for j in range(NT // 2):
                    bb_ref[slot, j * L + r0:j * L + r0 + rows] = jnp.concatenate(
                        tiles[2 * j:2 * j + 2], axis=1).astype(bf16)
                sums = [tiles[i] + tiles[j] + tiles[k]
                        for i, j, k in ((13, 15, 0), (27, 29, 2), (4, 6, 8), (18, 20, 22))]
                marks += [t[8 * c:8 * c + 8] for c in range(rows // 8) for t in sums]
            xr = (load(s, q, KM, KR) - mean) * rstd
            for j in range(2):
                bb_ref[slot, RO + j * KR:RO + (j + 1) * KR] = xr[:, 2 * j * L:(2 * j + 2) * L].astype(bf16)
            t = xr[:, :L] + xr[:, L:2 * L] + xr[:, 2 * L:3 * L] + xr[:, 3 * L:]
            return marks + [t[8 * c:8 * c + 8] for c in range(KR // 8)]

        def mm(s, q, slot, gates, never, done):
            def lhs(ref, key):
                t = ref[...]
                nr = t.shape[0] // 8
                runs, j = [], 0
                while j < nr:
                    e = j
                    while e < nr and ((key, e) in gates) == ((key, j) in gates):
                        e += 1
                    v = t[8 * j:8 * e]
                    if (key, j) in gates:
                        v = jnp.where(never(e - j),
                                      jnp.concatenate([gates[key, i] for i in range(j, e)], axis=0), v)
                    runs.append(v)
                    j = e
                return pltpu.bitcast(jnp.concatenate(runs, axis=0), bf16)

            def tile(t):
                return bb_ref[slot, (t // 2) * L:(t // 2 + 1) * L, (t % 2) * L:(t % 2 + 1) * L]

            def rem(t):
                return bb_ref[slot, RO + (t // 2) * KR:RO + (t // 2 + 1) * KR, (t % 2) * L:(t % 2 + 1) * L]

            def dot(p, r):
                return jnp.dot(p, r, preferred_element_type=f32)

            def one_level(i, grp, cols):
                l = jnp.concatenate([lhs(al_ref.at[i, kt], ('l', grp, kt)) for kt in range(2)], axis=1)
                t0 = (0, 32, 36)[i]
                return [dot(l, jnp.concatenate([tile(t0 + 2 * j), tile(t0 + 2 * j + 1)], axis=0)) for j in cols]

            m0 = one_level(0, 0, (0, 1))
            acc = {}
            for h in range(2):
                for j in range(2):
                    st_ref[2, :, :L] = jnp.zeros((8, L), f32)
                    p, = one_level(1 + h, 1 + 2 * h + j, (j,))
                    l = pltpu.bitcast(ar_ref[h], bf16)[:, :KR]
                    bias = c_ref[h * MH:(h + 1) * MH]
                    diag = ((p - m0[j]) if h else (p + m0[j])) + dot(l, rem(2 * h + j)) + bias
                    off = dot(l, rem(2 * (1 - h) + j)) + bias
                    acc[h, h, j] = [diag[:MQ], diag[MQ:]]
                    acc[h, 1 - h, j] = [off[:MQ], off[MQ:]]

            def two_level(i, dests):
                part = {}
                left = {k: len(v) for k, v in _COMB.items()}
                for p in _PORD[i]:
                    r = dot(lhs(as_ref.at[i, p], ('s', i, p)), tile(4 + 7 * i + p))
                    for k, terms in _COMB.items():
                        for sg in [sg for pp, sg in terms if pp == p]:
                            if k in part:
                                v, s0 = part[k]
                                part[k] = ((v + r) if sg == s0 else (v - r), s0)
                            else:
                                part[k] = (r, sg)
                            left[k] -= 1
                            if not left[k]:
                                v, s0 = part[k]
                                for h, th in dests:
                                    dst = acc[h, th, (1 - k[1]) if _SWAP[i] else k[1]]
                                    dst[k[0]] = (dst[k[0]] + v) if s0 > 0 else (dst[k[0]] - v)

            def emit(h, th):
                c0 = q * QT + th * 2 * L
                obuf[s, h * MH:(h + 1) * MH, c0:c0 + 2 * L] = jnp.concatenate(
                    [jnp.concatenate(acc[h, th, j], axis=0) for j in range(2)], axis=1).astype(bf16)

            two_level(0, ((1, 0), (1, 1)))
            two_level(1, ((0, 0), (1, 0)))
            emit(1, 0)
            done(slice(MH, D), 0)
            two_level(2, ((0, 0), (0, 1)))
            emit(0, 0)
            done(slice(0, MH), 0)
            two_level(3, ((0, 1), (1, 1)))
            emit(0, 1)
            emit(1, 1)
            done(slice(0, D), 1)

        def block(sbase, u0, n, h, never, done=lambda u, rows, th: None, lag=0):
            def loc(u):
                s = sbase + u // NQ
                return (s if u < u0 + n or isinstance(s, int) else jnp.minimum(s, S - 1)), u % NQ

            slots = [h] + list(range(2, n + 1)) + [1 - h]
            st = None if lag else (st_ref[h, 0:1], st_ref[h, 1:2])
            for j in range(n):
                u = u0 + j
                gates = {}
                if lag:
                    st, marks = stats(*loc(u + 1))
                    gates.update(zip(stat_h, marks, strict=True))
                    st_ref[2, 0:1] = st[0]
                gates.update(zip(norm_h if lag else norm_at,
                                 norm(*loc(u + 1), slots[j + 1], *st), strict=True))
                if lag < 2:
                    st, marks = stats(*loc(u + 2))
                    gates.update(zip(stat_h2 if lag else stat_at, marks, strict=True))
                mm(*loc(u), slots[j], gates, never, lambda rows, th, u=u: done(u, rows, th))
            if lag < 2:
                st_ref[1 - h, 0:1] = st[0]
                st_ref[1 - h, 1:2] = st[1]

        def never_from(zero):
            return lambda nr: jax.lax.broadcasted_iota(jnp.int32, (8 * nr, L), 1) < zero

        e = c_ref[0:8][0, 0]
        never0 = never_from(jnp.logical_and(e > 0, e < 0).astype(jnp.int32))
        head_copy(0).wait()
        norm(0, 0, 0, *stats(0, 0, rows=64)[0], rows=8)
        u, waited = 0, 1
        for bi, n in enumerate(HEAD):
            need = 2 if bi == 0 else u + n + 2
            for j in range(waited, need):
                head_copy(j).wait()
            block(0, u, n, bi % 2, never0, lag=max(2 - bi, 0))
            u, waited = u + n, need
        assert waited == NH

        @pl.loop(0, NIT)
        def _(i):
            never = never_from(jax.lax.shift_right_logical(i, 10))
            for hh in range(2):
                if hh == 0:
                    grp_copy(i, 0).wait()
                else:
                    pl.when(i < NIT - 1)(lambda: grp_copy(i, 1).wait())
                    pl.when(i == NIT - 1)(lambda: grp_copy(i, 1, True).wait())
                if WSB % 2 == hh:
                    pl.when(i == WSB // 2)(
                        lambda: out_slices(0, ((WSB // 2) * UI + BOFF[hh]) // NQ).start())

                def done(u, rows, th):
                    c0 = (u % NQ) * QT
                    cond = 2 * i + hh >= WSB
                    if u >= U0 + UI - NQ:
                        pl.when(i == NIT - 1)(
                            lambda: out_part(S - 1, rows, c0 + th * 2 * L, 2 * L).start())
                        cond = jnp.logical_and(cond, i < NIT - 1)
                    if th:
                        pl.when(cond)(lambda: out_part(i * SI + u // NQ, slice(0, D), c0, QT).start())

                block(i * SI, BOFF[hh], BUS[hh], (len(HEAD) + hh) % 2, never, done)

        out_slices(0, S).wait()

    out = pl.pallas_call(
        kernel,
        in_specs=[pl.BlockSpec(memory_space=pl.ANY)] * 4,
        out_specs=pl.BlockSpec(memory_space=pl.ANY),
        out_shape=jax.ShapeDtypeStruct((S, D, B), x.dtype),
        scratch_shapes=[pltpu.VMEM((S, D, B), bf16),
                        pltpu.VMEM((S, D, B), bf16),
                        pltpu.VMEM((D, D), bf16),
                        pltpu.VMEM((D,), bf16),
                        pltpu.VMEM((D,), bf16),
                        pltpu.VMEM((3, 2, MH // 2, L), f32),
                        pltpu.VMEM((4, 7, MQ // 2, L), f32),
                        pltpu.VMEM((2, MH // 2, L), f32),
                        pltpu.VMEM((D, L), f32),
                        pltpu.VMEM((max(BUS + HEAD) + 1, RO + 2 * KR, 2 * L), bf16),
                        pltpu.VMEM((3, 8, QT), f32),
                        pltpu.SemaphoreType.DMA((NH,)),
                        pltpu.SemaphoreType.DMA((2 * NIT,)),
                        pltpu.SemaphoreType.DMA(()),
                        pltpu.SemaphoreType.DMA((3,))],
        compiler_params=pltpu.CompilerParams(
            vmem_limit_bytes=110 * 1024 * 1024,
            disable_bounds_checks=True, disable_semaphore_checks=True),
    )(jnp.transpose(x, (1, 2, 0)), g, b, w)
    return jnp.transpose(out, (2, 0, 1))
```
